```python
import os as _os
_os.environ.setdefault("JAX_PLATFORMS", "cpu")
import jax
import jax.numpy as jnp

def _softmax(x, axis=-1):
    return jax.nn.softmax(x, axis=axis)
def _gelu(x):
    return jax.nn.gelu(x, approximate=True)
def _silu(x):
    return jax.nn.silu(x)
def _sigmoid(x):
    return jax.nn.sigmoid(x)
def _layernorm(x, axis=-1, eps=1e-5):
    m = jnp.mean(x, axis=axis, keepdims=True)
    v = jnp.var(x, axis=axis, keepdims=True)
    return (x - m) / jnp.sqrt(v + eps)
def _scatter_add(tgt, idx, src, axis=0):
    return tgt.at[idx].add(src)
def _segment_sum(src, seg, n):
    return jax.ops.segment_sum(src, seg, n)
class _Rng:
    def __init__(self, key):
        self._k = key
    def _next(self):
        self._k, sub = jax.random.split(self._k)
        return sub
    def normal(self, shape):
        return jax.random.normal(self._next(), shape, dtype=jnp.bfloat16)
    def randint(self, lo, hi, shape):
        return jax.random.randint(self._next(), shape, lo, hi, dtype=jnp.int32)
    def uniform(self, shape, lo=0.0, hi=1.0):
        return jax.random.uniform(self._next(), shape, jnp.bfloat16, lo, hi)
    def permutation(self, n):
        return jax.random.permutation(self._next(), n)


kernel_name = 'gated_mix__ssm_conv_s5__glu_gated_geglu__prompt'

def setup_inputs():
    _rng = _Rng(jax.random.key(int.from_bytes(__import__("os").urandom(4), "little")))
    _w = (lambda a: (lambda t: t.astype(jnp.bfloat16) if jnp.issubdtype(t.dtype, jnp.floating) else t)(jnp.asarray(a)))
    def _A_setup():
        B, S, D = 1, 2048, 448
        P = D
        Lambda_re = -0.5 * jnp.exp((lambda *s: _rng.normal(s) * 0.4)(P))
        Lambda_im = (lambda *s: _rng.normal(s) * 0.4)(P) * 1.0
        B_re = (lambda *s: _rng.normal(s) * 0.4)(P, D) * (D ** -0.5)
        B_im = (lambda *s: _rng.normal(s) * 0.4)(P, D) * (D ** -0.5)
        C_re = (lambda *s: _rng.normal(s) * 0.4)(D, P) * (P ** -0.5)
        C_im = (lambda *s: _rng.normal(s) * 0.4)(D, P) * (P ** -0.5)
        log_dt = (lambda *s: _rng.normal(s) * 0.4)(P) * 0.3 - 2.0
        Dskip = (lambda *s: _rng.normal(s) * 0.4)(D)
        return {
            "x": _w((lambda *s: _rng.normal(s) * 0.05)(B, S, D)),
            "Lambda_re": _w(Lambda_re),
            "Lambda_im": _w(Lambda_im),
            "B_re": _w(B_re),
            "B_im": _w(B_im),
            "C_re": _w(C_re),
            "C_im": _w(C_im),
            "log_dt": _w(log_dt),
            "Dskip": _w(Dskip),
        }
    _A_in = _A_setup()

    def _B_setup():
        B, S, Dm, Df = 1, 2048, 448, 1792
        return {
            "x": _w((lambda *s: _rng.normal(s) * 0.05)(B, S, Dm)),
            "w_gate": _w((lambda *s: _rng.normal(s) * 1.6)(Dm, Df) * (Dm ** -0.5)),
            "w_up": _w((lambda *s: _rng.normal(s) * 1.6)(Dm, Df) * (Dm ** -0.5)),
            "w_down": _w((lambda *s: _rng.normal(s) * 1.6)(Df, Dm) * (Df ** -0.5)),
        }
    _B_in = _B_setup()

    return {
        "A_x": _A_in["x"],
        "A_Lambda_re": _A_in["Lambda_re"],
        "A_Lambda_im": _A_in["Lambda_im"],
        "A_B_re": _A_in["B_re"],
        "A_B_im": _A_in["B_im"],
        "A_C_re": _A_in["C_re"],
        "A_C_im": _A_in["C_im"],
        "A_log_dt": _A_in["log_dt"],
        "A_Dskip": _A_in["Dskip"],
        "B_x": _B_in["x"],
        "B_w_gate": _B_in["w_gate"],
        "B_w_up": _B_in["w_up"],
        "B_w_down": _B_in["w_down"],
        "gate_w": _w((lambda *s: _rng.normal(s) * 0.05)(448) * 16.0),
    }

def reference(A_x, A_Lambda_re, A_Lambda_im, A_B_re, A_B_im, A_C_re, A_C_im, A_log_dt, A_Dskip, B_x, B_w_gate, B_w_up, B_w_down, gate_w):
    def _A_ref(x, Lambda_re, Lambda_im, B_re, B_im, C_re, C_im, log_dt, Dskip):
        Bsz, L, H = x.shape
        Lam = Lambda_re + 1j * Lambda_im
        Bmat = B_re + 1j * B_im
        Cmat = C_re + 1j * C_im
        dt = jnp.exp(log_dt)
        Lam_bar = jnp.exp(dt * Lam)
        B_bar = ((Lam_bar - 1.0) / Lam)[:, None] * Bmat
        Bu = jnp.einsum("bld,pd->blp", x + 0j, B_bar)
        h = jnp.zeros_like(Bu[:, 0, :])
        hs = []
        for t in range(L):
            h = Lam_bar[None, :] * h + Bu[:, t, :]
            hs.append(h)
        hseq = jnp.stack(hs, 1)
        y = 2.0 * jnp.einsum("blp,dp->bld", hseq, Cmat).real + x * Dskip[None, None, :]
        return y

    def _B_ref(x, w_gate, w_up, w_down):
        g = jnp.einsum("bsd,df->bsf", x, w_gate)
        u = jnp.einsum("bsd,df->bsf", x, w_up)
        h = _gelu(g) * u
        return jnp.einsum("bsf,fd->bsd", h, w_down)

    x = A_x
    g = _sigmoid((x * gate_w).sum(-1, keepdims=True))
    a = _A_ref(x, A_Lambda_re, A_Lambda_im, A_B_re, A_B_im, A_C_re, A_C_im, A_log_dt, A_Dskip)
    b = _B_ref(x, B_w_gate, B_w_up, B_w_down)
    return g * a + (1 - g) * b
```

```python
import numpy as np
import jax
import jax.numpy as jnp
import jax.experimental.pallas as pl
import jax.experimental.pallas.tpu as pltpu

F32 = jnp.float32
BF16 = jnp.bfloat16
I32 = jnp.int32

NN = (((1,), (0,)), ((), ()))
NT = (((1,), (1,)), ((), ()))

LANES = 128
SEG = 16
HR = LANES // 2
CT = 2
X_PIECES = (2, 4, 10)
FFN_BLOCKS = (128, 640, 512, 512)
FFN_UNROLL = 4


def _cmul(ar, ai, br, bi):
    return ar * br - ai * bi, ar * bi + ai * br


def _gelu(x):
    c0 = np.float32(np.sqrt(2.0 / np.pi))
    c1 = np.float32(np.sqrt(2.0 / np.pi) * 0.044715)
    hx = 0.5 * x
    return hx + hx * jnp.tanh(x * (c0 + c1 * (x * x)))


def _make_kernel(T, D, P, F):
    NTL = T // LANES
    M = CT * LANES
    NCH = T // M
    PF = (P // LANES) * LANES
    PH = P - PF
    W = PF + LANES
    P2 = 2 * P
    NBO = [int(v) for v in np.cumsum((0,) + FFN_BLOCKS)]
    NJ = len(FFN_BLOCKS)
    assert PH == LANES // 2 and D % 16 == 0 and NBO[-1] == F
    assert NTL == 16 and sum(X_PIECES) == NTL and NCH % FFN_UNROLL == 0

    def kernel(xT_hbm, lre_hbm, lim_hbm, bre_hbm, bim_hbm, cre_hbm, cim_hbm, ldt_hbm, dsk_hbm,
               wg_hbm, wu_hbm, wdT_hbm, gw_hbm,
               o_hbm,
               xT_s, bc_s, wg_s, wu_s, wd_s, cre_s, cim_s, cc_s, x_s, bu_s, h_s, out_s, dsk_s, gw_s,
               xp_s, par_s, hh_s, v0_s, v1_s, v2_s, v3_s, v4_s, sem, osem):
        v_s = (v0_s, v1_s, v2_s, v3_s, v4_s)
        cp_v = [pltpu.make_async_copy(src, dst, sem.at[i]) for i, (src, dst) in
                enumerate(zip((lre_hbm, lim_hbm, ldt_hbm, dsk_hbm, gw_hbm), v_s))]
        s0 = len(cp_v)
        xo = [int(v) * LANES for v in np.cumsum((0,) + X_PIECES)]
        cp_x = [pltpu.make_async_copy(xT_hbm.at[:, pl.ds(xo[i], xo[i + 1] - xo[i])],
                                      xT_s.at[:, pl.ds(xo[i], xo[i + 1] - xo[i])], sem.at[s0 + i])
                for i in range(len(X_PIECES))]
        s0 += len(cp_x)
        cp_b = [pltpu.make_async_copy(bre_hbm, bc_s.at[pl.ds(0, P)], sem.at[s0]),
                pltpu.make_async_copy(bim_hbm.at[pl.ds(PF, PH)], bc_s.at[pl.ds(P, PH)], sem.at[s0 + 1]),
                pltpu.make_async_copy(bim_hbm.at[pl.ds(0, PF)], bc_s.at[pl.ds(P + PH, PF)], sem.at[s0 + 2])]
        cp_w = [pltpu.make_async_copy(wg_hbm, wg_s, sem.at[s0 + 3]),
                pltpu.make_async_copy(wu_hbm, wu_s, sem.at[s0 + 4]),
                pltpu.make_async_copy(wdT_hbm, wd_s, sem.at[s0 + 5])]
        cp_c = [pltpu.make_async_copy(cre_hbm, cre_s, sem.at[s0 + 6]),
                pltpu.make_async_copy(cim_hbm, cim_s, sem.at[s0 + 7])]
        for c in cp_v + cp_x[:1] + cp_b + cp_x[1:] + cp_c + cp_w:
            c.start()

        def wait(copies):
            for c in copies:
                c.wait()

        sub = jax.lax.broadcasted_iota(I32, (8, W), 0)

        def params():
            wait(cp_v)

            def vec(i):
                return v_s[i][...].astype(F32).reshape(1, P)
            lam_r = jnp.broadcast_to(vec(0), (8, P))
            lam_i = jnp.broadcast_to(vec(1), (8, P))
            dt = jnp.broadcast_to(jnp.exp(vec(2)).astype(v2_s.dtype).astype(F32), (8, P))
            mag = jnp.exp(dt * lam_r)
            ang = dt * lam_i
            lb_r = mag * jnp.cos(ang)
            lb_i = mag * jnp.sin(ang)
            scale = jnp.maximum(jnp.abs(lam_r), jnp.abs(lam_i))
            ar = lam_r / scale
            ai = lam_i / scale
            den = (ar * ar + ai * ai) * scale
            nr = lb_r - 1.0
            co_r = (nr * ar + lb_i * ai) / den
            co_i = (lb_i * ar - nr * ai) / den

            lr = jnp.concatenate([lb_r, lb_r[:, PF:P]], axis=1)
            li = jnp.concatenate([lb_i, -lb_i[:, PF:P]], axis=1)
            pr, pi = lr, li
            for _ in range(4):
                pr, pi = _cmul(pr, pi, pr, pi)
            pw = [(pr, pi)]
            for _ in range(3):
                pw.append(_cmul(*pw[-1], *pw[-1]))
            lk_r = jnp.ones((8, W), F32)
            lk_i = jnp.zeros((8, W), F32)
            for b in range(3):
                tr, ti = _cmul(lk_r, lk_i, *pw[b])
                m = (sub & (1 << b)) != 0
                lk_r = jnp.where(m, tr, lk_r)
                lk_i = jnp.where(m, ti, lk_i)
            for i, v in enumerate([lr, li] + [v for p in pw for v in p] + [lk_r, lk_i]):
                par_s[i] = v
            par_s[12, :, 0:P] = co_r * 2.0
            par_s[13, :, 0:P] = co_i * 2.0
            dsk_s[...] = jnp.broadcast_to(vec(3), (LANES, D)).T
            gw_s[...] = jnp.broadcast_to(vec(4), (LANES, D)).T

        lane_x = jax.lax.broadcasted_iota(I32, (D // 2, LANES), 1)
        fwd_idx = (lane_x % 8) * SEG + lane_x // 8

        def prep(m0, n):
            for m in range(m0, m0 + n):
                sl = slice(m * LANES, (m + 1) * LANES)
                xi = jnp.take_along_axis(pltpu.bitcast(xT_s[:, sl], I32), fwd_idx, axis=1)
                x_s[m * HR:(m + 1) * HR, :] = pltpu.bitcast(pltpu.bitcast(xi, BF16).T, I32)
                xp_s[:, sl] = xi

        def bu_mm(m0, n):
            xc = pltpu.bitcast(x_s[m0 * HR:(m0 + n) * HR, :], BF16)
            bu_s[m0 * LANES:(m0 + n) * LANES, :] = jax.lax.dot_general(
                xc, bc_s[...], NT, preferred_element_type=F32)

        carry = [[None] * (W // LANES), [None] * (W // LANES)]

        def scan_tile(m):
            r0 = m * LANES
            sub1 = sub[:, 0:LANES]
            for k in range(W // LANES):
                cs = slice(k * LANES, (k + 1) * LANES)
                ci = slice(W + k * LANES, W + (k + 1) * LANES)
                half = k == W // LANES - 1

                def par(i):
                    return par_s[i, :, cs]

                def ld(j):
                    br = bu_s[r0 + 8 * j:r0 + 8 * j + 8, cs]
                    bi = pltpu.roll(br, 64, 1) if half else bu_s[r0 + 8 * j:r0 + 8 * j + 8, ci]
                    return br, bi
                lr, li = par(0), par(1)
                hr, hi = ld(0)
                for j in range(1, SEG):
                    br, bi = ld(j)
                    tr, ti = _cmul(lr, li, hr, hi)
                    hr, hi = tr + br, ti + bi
                sr, si = hr, hi
                for b in range(3):
                    d = 1 << b
                    tr, ti = _cmul(par(2 + 2 * b), par(3 + 2 * b),
                                   pltpu.roll(sr, d, 0), pltpu.roll(si, d, 0))
                    sr = jnp.where(sub1 >= d, sr + tr, sr)
                    si = jnp.where(sub1 >= d, si + ti, si)
                hr = jnp.where(sub1 >= 1, pltpu.roll(sr, 1, 0), 0.0)
                hi = jnp.where(sub1 >= 1, pltpu.roll(si, 1, 0), 0.0)
                nr = jnp.broadcast_to(sr[7:8, :], (8, LANES))
                ni = jnp.broadcast_to(si[7:8, :], (8, LANES))
                if carry[0][k] is not None:
                    tr, ti = _cmul(par(10), par(11), carry[0][k], carry[1][k])
                    hr, hi = hr + tr, hi + ti
                    tr, ti = _cmul(par(8), par(9), carry[0][k], carry[1][k])
                    nr, ni = nr + tr, ni + ti
                carry[0][k], carry[1][k] = nr, ni
                prev = None
                for j in range(SEG):
                    br, bi = ld(j)
                    tr, ti = _cmul(lr, li, hr, hi)
                    hr, hi = tr + br, ti + bi
                    if j % 2 == 1:
                        rs = slice(m * HR + 4 * (j - 1), m * HR + 4 * (j + 1))
                        h_s[rs, cs] = pltpu.bitcast(
                            jnp.concatenate([prev[0], hr], axis=0).astype(BF16), I32)
                        if not half:
                            h_s[rs, ci] = pltpu.bitcast(
                                jnp.concatenate([prev[1], hi], axis=0).astype(BF16), I32)
                    prev = (hr, hi)

        def scan(m0, n):
            for m in range(m0, m0 + n):
                scan_tile(m)

        def build_c():
            cr = par_s[12, 0:1, 0:P]
            ci = par_s[13, 0:1, 0:P]
            for r in range(0, D, 16):
                a = cre_s[r:r + 16, :].astype(F32)
                b = cim_s[r:r + 16, :].astype(F32)
                re = a * cr - b * ci
                im = -(a * ci) - b * cr
                cat = jnp.concatenate([re, im[:, PF:P], im[:, 0:PF]], axis=1)
                cc_s[r // 2:r // 2 + 8, :] = pltpu.bitcast(cat.astype(BF16), I32)

        def y_mm(m0, n):
            hc = pltpu.bitcast(h_s[m0 * HR:(m0 + n) * HR, :], BF16)
            out_s[:, m0 * LANES:(m0 + n) * LANES] = jax.lax.dot_general(
                pltpu.bitcast(cc_s[...], BF16), hc, NT, preferred_element_type=F32)

        def up(xc, j):
            g = jax.lax.dot_general(xc, wg_s[:, NBO[j]:NBO[j + 1]], NN, preferred_element_type=F32)
            u = jax.lax.dot_general(xc, wu_s[:, NBO[j]:NBO[j + 1]], NN, preferred_element_type=F32)
            return (_gelu(g) * u).astype(BF16)

        def xchunk(c):
            return pltpu.bitcast(x_s[pl.ds(pl.multiple_of(c * (M // 2), M // 2), M // 2), :], BF16)

        params()
        wait(cp_x[0:1])
        prep(0, 2)
        wait(cp_b)
        bu_mm(0, 1)
        wait(cp_x[1:2])
        prep(2, 4)
        bu_mm(1, 1)
        bu_mm(2, 2)
        scan(0, 1)
        bu_mm(4, 1)
        scan(1, 1)
        wait(cp_x[2:3])
        wait(cp_c)
        build_c()
        prep(6, 10)
        bu_mm(5, 1)
        for m in range(6, NTL, 2):
            bu_mm(m, 2)
            scan(m - 4, 2)
        y_mm(0, 4)
        scan(12, 2)
        y_mm(4, 4)
        scan(14, 2)
        y_mm(8, 4)
        wait(cp_w)
        y_mm(12, 4)
        hh_s[...] = pltpu.bitcast(up(xchunk(0), 0), I32)

        lane = jax.lax.broadcasted_iota(I32, (D, LANES), 1)
        inv_idx = 8 * (lane % SEG) + lane // SEG

        def gate(c0):
            acc = [None] * 4
            for k in range(D // 16):
                xf = pltpu.bitcast(xp_s[8 * k:8 * k + 8, pl.ds(c0, LANES)], BF16).astype(F32)
                pr = xf * gw_s[16 * k:16 * k + 16, :]
                pr = pr[0:8] + pr[8:16]
                acc[k % 4] = pr if acc[k % 4] is None else acc[k % 4] + pr
            return jax.nn.sigmoid(jnp.sum((acc[0] + acc[1]) + (acc[2] + acc[3]), axis=0, keepdims=True))

        def out_copy(m):
            c0 = pl.multiple_of(m * LANES, LANES)
            return pltpu.make_async_copy(out_s.at[:, pl.ds(c0, LANES)], o_hbm.at[:, pl.ds(c0, LANES)],
                                         osem.at[m])

        def chunk(c, _):
            xc = xchunk(c)
            hh = {0: pltpu.bitcast(hh_s[...], BF16)}
            bT = None
            for j in range(NJ - 1):
                hh[j + 1] = up(xc, j + 1)
                d = jax.lax.dot_general(wd_s[:, NBO[j]:NBO[j + 1]], hh.pop(j), NT,
                                        preferred_element_type=F32)
                bT = d if bT is None else bT + d
            h_last = hh.pop(NJ - 1)
            bs = []
            for t in range(CT):
                ts = slice(t * LANES, (t + 1) * LANES)
                bs.append(bT[:, ts] + jax.lax.dot_general(wd_s[:, NBO[NJ - 1]:F], h_last[ts, :], NT,
                                                          preferred_element_type=F32))
            hh_s[...] = pltpu.bitcast(up(xchunk(jnp.minimum(c + 1, NCH - 1)), 0), I32)
            for t in range(CT):
                c0 = pl.multiple_of(c * M + t * LANES, LANES)
                g = gate(c0)
                xf = pltpu.bitcast(xp_s[:, pl.ds(c0, LANES)], BF16).astype(F32)
                b = bs[t]
                a = out_s[:, pl.ds(c0, LANES)] + xf * dsk_s[...]
                out_s[:, pl.ds(c0, LANES)] = jnp.take_along_axis(b + g * (a - b), inv_idx, axis=1)
                out_copy(c * CT + t).start()
            return _

        jax.lax.fori_loop(0, NCH, chunk, 0, unroll=FFN_UNROLL)
        for m in range(NTL):
            out_copy(m).wait()

    return kernel


@jax.jit
def pallas_gated_mix__ssm_conv_s5__glu_gated_geglu__prompt_kernel(
    A_x: jax.Array,
    A_Lambda_re: jax.Array,
    A_Lambda_im: jax.Array,
    A_B_re: jax.Array,
    A_B_im: jax.Array,
    A_C_re: jax.Array,
    A_C_im: jax.Array,
    A_log_dt: jax.Array,
    A_Dskip: jax.Array,
    B_x: jax.Array,
    B_w_gate: jax.Array,
    B_w_up: jax.Array,
    B_w_down: jax.Array,
    gate_w: jax.Array,
):
    del B_x
    _, T, D = A_x.shape
    P = A_B_re.shape[0]
    F = B_w_gate.shape[1]
    any_spec = pl.BlockSpec(memory_space=pl.ANY)
    out_t = pl.pallas_call(
        _make_kernel(T, D, P, F),
        out_shape=jax.ShapeDtypeStruct((D, T), F32),
        in_specs=[any_spec] * 13,
        out_specs=any_spec,
        scratch_shapes=[
            pltpu.VMEM((D, T), BF16),
            pltpu.VMEM((2 * P, D), BF16),
            pltpu.VMEM((D, F), BF16),
            pltpu.VMEM((D, F), BF16),
            pltpu.VMEM((D, F), BF16),
            pltpu.VMEM((D, P), BF16),
            pltpu.VMEM((D, P), BF16),
            pltpu.VMEM((D // 2, 2 * P), I32),
            pltpu.VMEM((T // 2, D), I32),
            pltpu.VMEM((T, 2 * P), F32),
            pltpu.VMEM((T // 2, 2 * P), I32),
            pltpu.VMEM((D, T), F32),
            pltpu.VMEM((D, LANES), F32),
            pltpu.VMEM((D, LANES), F32),
            pltpu.VMEM((D // 2, T), I32),
            pltpu.VMEM((14, 8, P + P % LANES), F32),
            pltpu.VMEM((CT * HR, FFN_BLOCKS[0]), I32),
            *[pltpu.VMEM((P,), v.dtype) for v in (A_Lambda_re, A_Lambda_im, A_log_dt, A_Dskip, gate_w)],
            pltpu.SemaphoreType.DMA((5 + len(X_PIECES) + 8,)),
            pltpu.SemaphoreType.DMA((T // LANES,)),
        ],
        compiler_params=pltpu.CompilerParams(
            vmem_limit_bytes=100 * 1024 * 1024,
            disable_bounds_checks=True,
            disable_semaphore_checks=True,
        ),
        name="gated_mix_s5_geglu",
    )(A_x[0].T, A_Lambda_re, A_Lambda_im, A_B_re, A_B_im, A_C_re, A_C_im, A_log_dt, A_Dskip,
      B_w_gate, B_w_up, B_w_down.T, gate_w)
    return out_t.T[None]
```

```python
import numpy as np
import jax
import jax.numpy as jnp
import jax.experimental.pallas as pl
import jax.experimental.pallas.tpu as pltpu

F32 = jnp.float32
BF16 = jnp.bfloat16
I32 = jnp.int32

NN = (((1,), (0,)), ((), ()))
NT = (((1,), (1,)), ((), ()))

LANES = 128
SEG = 16
HR = LANES // 2
CT = 2
X_PIECES = (2, 5, 9)
FFN_BLOCKS = (128, 640, 512, 512)
FFN_UNROLL = 4


def _cmul(ar, ai, br, bi):
    return ar * br - ai * bi, ar * bi + ai * br


def _gelu(x):
    c0 = np.float32(np.sqrt(2.0 / np.pi))
    c1 = np.float32(np.sqrt(2.0 / np.pi) * 0.044715)
    hx = 0.5 * x
    return hx + hx * jnp.tanh(x * (c0 + c1 * (x * x)))


def _make_kernel(T, D, P, F):
    NTL = T // LANES
    M = CT * LANES
    NCH = T // M
    PF = (P // LANES) * LANES
    PH = P - PF
    W = PF + LANES
    P2 = 2 * P
    NBO = [int(v) for v in np.cumsum((0,) + FFN_BLOCKS)]
    NJ = len(FFN_BLOCKS)
    assert PH == LANES // 2 and D % 16 == 0 and NBO[-1] == F
    assert NTL == 16 and sum(X_PIECES) == NTL and NCH % FFN_UNROLL == 0

    def kernel(xT_hbm, lre_hbm, lim_hbm, bre_hbm, bim_hbm, cre_hbm, cim_hbm, ldt_hbm, dsk_hbm,
               wg_hbm, wu_hbm, wdT_hbm, gw_hbm,
               o_hbm,
               xT_s, bc_s, wg_s, wu_s, wd_s, cre_s, cim_s, cc_s, x_s, bu_s, h_s, out_s, dsk_s, gw_s,
               xp_s, par_s, hh_s, v0_s, v1_s, v2_s, v3_s, v4_s, sem, osem):
        v_s = (v0_s, v1_s, v2_s, v3_s, v4_s)
        cp_v = [pltpu.make_async_copy(src, dst, sem.at[i]) for i, (src, dst) in
                enumerate(zip((lre_hbm, lim_hbm, ldt_hbm, dsk_hbm, gw_hbm), v_s))]
        s0 = len(cp_v)
        xo = [int(v) * LANES for v in np.cumsum((0,) + X_PIECES)]
        cp_x = [pltpu.make_async_copy(xT_hbm.at[:, pl.ds(xo[i], xo[i + 1] - xo[i])],
                                      xT_s.at[:, pl.ds(xo[i], xo[i + 1] - xo[i])], sem.at[s0 + i])
                for i in range(len(X_PIECES))]
        s0 += len(cp_x)
        cp_b = [pltpu.make_async_copy(bre_hbm, bc_s.at[pl.ds(0, P)], sem.at[s0]),
                pltpu.make_async_copy(bim_hbm.at[pl.ds(PF, PH)], bc_s.at[pl.ds(P, PH)], sem.at[s0 + 1]),
                pltpu.make_async_copy(bim_hbm.at[pl.ds(0, PF)], bc_s.at[pl.ds(P + PH, PF)], sem.at[s0 + 2])]
        cp_w = [pltpu.make_async_copy(wg_hbm, wg_s, sem.at[s0 + 3]),
                pltpu.make_async_copy(wu_hbm, wu_s, sem.at[s0 + 4]),
                pltpu.make_async_copy(wdT_hbm, wd_s, sem.at[s0 + 5])]
        cp_c = [pltpu.make_async_copy(cre_hbm, cre_s, sem.at[s0 + 6]),
                pltpu.make_async_copy(cim_hbm, cim_s, sem.at[s0 + 7])]
        for c in cp_v + cp_x[:1] + cp_b + cp_x[1:] + cp_c + cp_w:
            c.start()

        def wait(copies):
            for c in copies:
                c.wait()

        sub = jax.lax.broadcasted_iota(I32, (8, W), 0)

        def params():
            wait(cp_v)

            def vec(i):
                return v_s[i][...].astype(F32).reshape(1, P)
            lam_r = jnp.broadcast_to(vec(0), (8, P))
            lam_i = jnp.broadcast_to(vec(1), (8, P))
            dt = jnp.broadcast_to(jnp.exp(vec(2)).astype(v2_s.dtype).astype(F32), (8, P))
            mag = jnp.exp(dt * lam_r)
            ang = dt * lam_i
            lb_r = mag * jnp.cos(ang)
            lb_i = mag * jnp.sin(ang)
            scale = jnp.maximum(jnp.abs(lam_r), jnp.abs(lam_i))
            ar = lam_r / scale
            ai = lam_i / scale
            den = (ar * ar + ai * ai) * scale
            nr = lb_r - 1.0
            co_r = (nr * ar + lb_i * ai) / den
            co_i = (lb_i * ar - nr * ai) / den

            lr = jnp.concatenate([lb_r, lb_r[:, PF:P]], axis=1)
            li = jnp.concatenate([lb_i, -lb_i[:, PF:P]], axis=1)
            pr, pi = lr, li
            for _ in range(4):
                pr, pi = _cmul(pr, pi, pr, pi)
            pw = [(pr, pi)]
            for _ in range(3):
                pw.append(_cmul(*pw[-1], *pw[-1]))
            lk_r = jnp.ones((8, W), F32)
            lk_i = jnp.zeros((8, W), F32)
            for b in range(3):
                tr, ti = _cmul(lk_r, lk_i, *pw[b])
                m = (sub & (1 << b)) != 0
                lk_r = jnp.where(m, tr, lk_r)
                lk_i = jnp.where(m, ti, lk_i)
            for i, v in enumerate([lr, li] + [v for p in pw for v in p] + [lk_r, lk_i]):
                par_s[i] = v
            par_s[12, :, 0:P] = co_r * 2.0
            par_s[13, :, 0:P] = co_i * 2.0
            dsk_s[...] = jnp.broadcast_to(vec(3), (LANES, D)).T
            gw_s[...] = jnp.broadcast_to(vec(4), (LANES, D)).T

        lane_x = jax.lax.broadcasted_iota(I32, (D // 2, LANES), 1)
        fwd_idx = (lane_x % 8) * SEG + lane_x // 8

        def prep(m0, n):
            for m in range(m0, m0 + n):
                sl = slice(m * LANES, (m + 1) * LANES)
                xi = jnp.take_along_axis(pltpu.bitcast(xT_s[:, sl], I32), fwd_idx, axis=1)
                x_s[m * HR:(m + 1) * HR, :] = pltpu.bitcast(pltpu.bitcast(xi, BF16).T, I32)
                xp_s[:, sl] = xi

        def bu_mm(m0, n):
            xc = pltpu.bitcast(x_s[m0 * HR:(m0 + n) * HR, :], BF16)
            bu_s[m0 * LANES:(m0 + n) * LANES, :] = jax.lax.dot_general(
                xc, bc_s[...], NT, preferred_element_type=F32)

        carry = [[None] * (W // LANES), [None] * (W // LANES)]

        def scan_tile(m):
            r0 = m * LANES
            sub1 = sub[:, 0:LANES]
            for k in range(W // LANES):
                cs = slice(k * LANES, (k + 1) * LANES)
                ci = slice(W + k * LANES, W + (k + 1) * LANES)
                half = k == W // LANES - 1

                def par(i):
                    return par_s[i, :, cs]

                def ld(j):
                    br = bu_s[r0 + 8 * j:r0 + 8 * j + 8, cs]
                    bi = pltpu.roll(br, 64, 1) if half else bu_s[r0 + 8 * j:r0 + 8 * j + 8, ci]
                    return br, bi
                lr, li = par(0), par(1)
                hr, hi = ld(0)
                for j in range(1, SEG):
                    br, bi = ld(j)
                    tr, ti = _cmul(lr, li, hr, hi)
                    hr, hi = tr + br, ti + bi
                sr, si = hr, hi
                for b in range(3):
                    d = 1 << b
                    tr, ti = _cmul(par(2 + 2 * b), par(3 + 2 * b),
                                   pltpu.roll(sr, d, 0), pltpu.roll(si, d, 0))
                    sr = jnp.where(sub1 >= d, sr + tr, sr)
                    si = jnp.where(sub1 >= d, si + ti, si)
                hr = jnp.where(sub1 >= 1, pltpu.roll(sr, 1, 0), 0.0)
                hi = jnp.where(sub1 >= 1, pltpu.roll(si, 1, 0), 0.0)
                nr = jnp.broadcast_to(sr[7:8, :], (8, LANES))
                ni = jnp.broadcast_to(si[7:8, :], (8, LANES))
                if carry[0][k] is not None:
                    tr, ti = _cmul(par(10), par(11), carry[0][k], carry[1][k])
                    hr, hi = hr + tr, hi + ti
                    tr, ti = _cmul(par(8), par(9), carry[0][k], carry[1][k])
                    nr, ni = nr + tr, ni + ti
                carry[0][k], carry[1][k] = nr, ni
                prev = None
                for j in range(SEG):
                    br, bi = ld(j)
                    tr, ti = _cmul(lr, li, hr, hi)
                    hr, hi = tr + br, ti + bi
                    if j % 2 == 1:
                        rs = slice(m * HR + 4 * (j - 1), m * HR + 4 * (j + 1))
                        h_s[rs, cs] = pltpu.bitcast(
                            jnp.concatenate([prev[0], hr], axis=0).astype(BF16), I32)
                        if not half:
                            h_s[rs, ci] = pltpu.bitcast(
                                jnp.concatenate([prev[1], hi], axis=0).astype(BF16), I32)
                    prev = (hr, hi)

        def scan(m0, n):
            for m in range(m0, m0 + n):
                scan_tile(m)

        def build_c():
            cr = par_s[12, 0:1, 0:P]
            ci = par_s[13, 0:1, 0:P]
            for r in range(0, D, 16):
                a = cre_s[r:r + 16, :].astype(F32)
                b = cim_s[r:r + 16, :].astype(F32)
                re = a * cr - b * ci
                im = -(a * ci) - b * cr
                cat = jnp.concatenate([re, im[:, PF:P], im[:, 0:PF]], axis=1)
                cc_s[r // 2:r // 2 + 8, :] = pltpu.bitcast(cat.astype(BF16), I32)

        def y_mm(m0, n):
            hc = pltpu.bitcast(h_s[m0 * HR:(m0 + n) * HR, :], BF16)
            out_s[:, m0 * LANES:(m0 + n) * LANES] = jax.lax.dot_general(
                pltpu.bitcast(cc_s[...], BF16), hc, NT, preferred_element_type=F32)

        def up(xc, j):
            g = jax.lax.dot_general(xc, wg_s[:, NBO[j]:NBO[j + 1]], NN, preferred_element_type=F32)
            u = jax.lax.dot_general(xc, wu_s[:, NBO[j]:NBO[j + 1]], NN, preferred_element_type=F32)
            return (_gelu(g) * u).astype(BF16)

        def xchunk(c):
            return pltpu.bitcast(x_s[pl.ds(pl.multiple_of(c * (M // 2), M // 2), M // 2), :], BF16)

        params()
        wait(cp_x[0:1])
        prep(0, 2)
        wait(cp_b)
        bu_mm(0, 1)
        wait(cp_x[1:2])
        prep(2, 5)
        bu_mm(1, 1)
        bu_mm(2, 2)
        scan(0, 1)
        bu_mm(4, 1)
        scan(1, 1)
        wait(cp_x[2:3])
        wait(cp_c)
        build_c()
        prep(7, 9)
        bu_mm(5, 2)
        scan(2, 2)
        bu_mm(7, 1)
        for m in range(8, NTL, 2):
            bu_mm(m, 2)
            scan(m - 4, 2)
        y_mm(0, 4)
        scan(12, 2)
        y_mm(4, 4)
        scan(14, 2)
        y_mm(8, 4)
        wait(cp_w)
        y_mm(12, 4)
        hh_s[...] = pltpu.bitcast(up(xchunk(0), 0), I32)

        lane = jax.lax.broadcasted_iota(I32, (D, LANES), 1)
        inv_idx = 8 * (lane % SEG) + lane // SEG

        def gate(c0):
            acc = [None] * 4
            for k in range(D // 16):
                xf = pltpu.bitcast(xp_s[8 * k:8 * k + 8, pl.ds(c0, LANES)], BF16).astype(F32)
                pr = xf * gw_s[16 * k:16 * k + 16, :]
                pr = pr[0:8] + pr[8:16]
                acc[k % 4] = pr if acc[k % 4] is None else acc[k % 4] + pr
            return jax.nn.sigmoid(jnp.sum((acc[0] + acc[1]) + (acc[2] + acc[3]), axis=0, keepdims=True))

        def out_copy(m):
            c0 = pl.multiple_of(m * LANES, LANES)
            return pltpu.make_async_copy(out_s.at[:, pl.ds(c0, LANES)], o_hbm.at[:, pl.ds(c0, LANES)],
                                         osem.at[m])

        def chunk(c, _):
            xc = xchunk(c)
            hh = {0: pltpu.bitcast(hh_s[...], BF16)}
            bT = None
            for j in range(NJ - 1):
                hh[j + 1] = up(xc, j + 1)
                d = jax.lax.dot_general(wd_s[:, NBO[j]:NBO[j + 1]], hh.pop(j), NT,
                                        preferred_element_type=F32)
                bT = d if bT is None else bT + d
            h_last = hh.pop(NJ - 1)
            bs = []
            for t in range(CT):
                ts = slice(t * LANES, (t + 1) * LANES)
                bs.append(bT[:, ts] + jax.lax.dot_general(wd_s[:, NBO[NJ - 1]:F], h_last[ts, :], NT,
                                                          preferred_element_type=F32))
            hh_s[...] = pltpu.bitcast(up(xchunk(jnp.minimum(c + 1, NCH - 1)), 0), I32)
            for t in range(CT):
                c0 = pl.multiple_of(c * M + t * LANES, LANES)
                g = gate(c0)
                xf = pltpu.bitcast(xp_s[:, pl.ds(c0, LANES)], BF16).astype(F32)
                b = bs[t]
                a = out_s[:, pl.ds(c0, LANES)] + xf * dsk_s[...]
                out_s[:, pl.ds(c0, LANES)] = jnp.take_along_axis(b + g * (a - b), inv_idx, axis=1)
                out_copy(c * CT + t).start()
            return _

        jax.lax.fori_loop(0, NCH, chunk, 0, unroll=FFN_UNROLL)
        for m in range(NTL):
            out_copy(m).wait()

    return kernel


@jax.jit
def pallas_gated_mix__ssm_conv_s5__glu_gated_geglu__prompt_kernel(
    A_x: jax.Array,
    A_Lambda_re: jax.Array,
    A_Lambda_im: jax.Array,
    A_B_re: jax.Array,
    A_B_im: jax.Array,
    A_C_re: jax.Array,
    A_C_im: jax.Array,
    A_log_dt: jax.Array,
    A_Dskip: jax.Array,
    B_x: jax.Array,
    B_w_gate: jax.Array,
    B_w_up: jax.Array,
    B_w_down: jax.Array,
    gate_w: jax.Array,
):
    del B_x
    _, T, D = A_x.shape
    P = A_B_re.shape[0]
    F = B_w_gate.shape[1]
    any_spec = pl.BlockSpec(memory_space=pl.ANY)
    out_t = pl.pallas_call(
        _make_kernel(T, D, P, F),
        out_shape=jax.ShapeDtypeStruct((D, T), F32),
        in_specs=[any_spec] * 13,
        out_specs=any_spec,
        scratch_shapes=[
            pltpu.VMEM((D, T), BF16),
            pltpu.VMEM((2 * P, D), BF16),
            pltpu.VMEM((D, F), BF16),
            pltpu.VMEM((D, F), BF16),
            pltpu.VMEM((D, F), BF16),
            pltpu.VMEM((D, P), BF16),
            pltpu.VMEM((D, P), BF16),
            pltpu.VMEM((D // 2, 2 * P), I32),
            pltpu.VMEM((T // 2, D), I32),
            pltpu.VMEM((T, 2 * P), F32),
            pltpu.VMEM((T // 2, 2 * P), I32),
            pltpu.VMEM((D, T), F32),
            pltpu.VMEM((D, LANES), F32),
            pltpu.VMEM((D, LANES), F32),
            pltpu.VMEM((D // 2, T), I32),
            pltpu.VMEM((14, 8, P + P % LANES), F32),
            pltpu.VMEM((CT * HR, FFN_BLOCKS[0]), I32),
            *[pltpu.VMEM((P,), v.dtype) for v in (A_Lambda_re, A_Lambda_im, A_log_dt, A_Dskip, gate_w)],
            pltpu.SemaphoreType.DMA((5 + len(X_PIECES) + 8,)),
            pltpu.SemaphoreType.DMA((T // LANES,)),
        ],
        compiler_params=pltpu.CompilerParams(
            vmem_limit_bytes=100 * 1024 * 1024,
            disable_bounds_checks=True,
            disable_semaphore_checks=True,
        ),
        name="gated_mix_s5_geglu",
    )(A_x[0].T, A_Lambda_re, A_Lambda_im, A_B_re, A_B_im, A_C_re, A_C_im, A_log_dt, A_Dskip,
      B_w_gate, B_w_up, B_w_down.T, gate_w)
    return out_t.T[None]
```
